```python
import os as _os
_os.environ.setdefault("JAX_PLATFORMS", "cpu")
import jax
import jax.numpy as jnp

def _softmax(x, axis=-1):
    return jax.nn.softmax(x, axis=axis)
def _gelu(x):
    return jax.nn.gelu(x, approximate=True)
def _silu(x):
    return jax.nn.silu(x)
def _sigmoid(x):
    return jax.nn.sigmoid(x)
def _layernorm(x, axis=-1, eps=1e-5):
    m = jnp.mean(x, axis=axis, keepdims=True)
    v = jnp.var(x, axis=axis, keepdims=True)
    return (x - m) / jnp.sqrt(v + eps)
def _scatter_add(tgt, idx, src, axis=0):
    return tgt.at[idx].add(src)
def _segment_sum(src, seg, n):
    return jax.ops.segment_sum(src, seg, n)
class _Rng:
    def __init__(self, key):
        self._k = key
    def _next(self):
        self._k, sub = jax.random.split(self._k)
        return sub
    def normal(self, shape):
        return jax.random.normal(self._next(), shape, dtype=jnp.bfloat16)
    def randint(self, lo, hi, shape):
        return jax.random.randint(self._next(), shape, lo, hi, dtype=jnp.int32)
    def uniform(self, shape, lo=0.0, hi=1.0):
        return jax.random.uniform(self._next(), shape, jnp.bfloat16, lo, hi)
    def permutation(self, n):
        return jax.random.permutation(self._next(), n)


kernel_name = 'sequential_preLN__mha_block__mixer_token_mlp__prompt'

def setup_inputs():
    _rng = _Rng(jax.random.key(int.from_bytes(__import__("os").urandom(4), "little")))
    _w = (lambda a: (lambda t: t.astype(jnp.bfloat16) if jnp.issubdtype(t.dtype, jnp.floating) else t)(jnp.asarray(a)))
    def _A_setup():
        B, S, D, H = 1, 2048, 448, 16
        return {
            "x": _w((lambda *s: _rng.normal(s) * 0.05)(B, S, D)),
            "wqkv": _w((lambda *s: _rng.normal(s) * 0.05)(D, 3 * D)),
            "wo": _w((lambda *s: _rng.normal(s) * 0.05)(D, D)),
        }
    _A_in = _A_setup()

    def _B_setup():
        B, S, D, F = 1, 2048, 448, 1792
        return {
            "x": _w((lambda *s: _rng.normal(s) * 0.05)(B, S, D)),
            "w1": _w((lambda *s: _rng.normal(s) * 0.2)(S, F) * (S ** -0.5)),
            "b1": _w((lambda *s: _rng.normal(s) * 0.2)(F) * 0.02),
            "w2": _w((lambda *s: _rng.normal(s) * 0.2)(F, S) * (F ** -0.5)),
            "b2": _w((lambda *s: _rng.normal(s) * 0.05)(S) * 0.02),
        }
    _B_in = _B_setup()

    return {
        "A_x": _A_in["x"],
        "A_wqkv": _A_in["wqkv"],
        "A_wo": _A_in["wo"],
        "B_x": _B_in["x"],
        "B_w1": _B_in["w1"],
        "B_b1": _B_in["b1"],
        "B_w2": _B_in["w2"],
        "B_b2": _B_in["b2"],
    }

def reference(A_x, A_wqkv, A_wo, B_x, B_w1, B_b1, B_w2, B_b2):
    def _A_ref(x, wqkv, wo):
        B, S, D = x.shape
        H = 16
        Dh = D // H
        qkv = (lambda x, *d: x.transpose(*d))((x @ wqkv).reshape(B, S, 3, H, Dh), 2, 0, 3, 1, 4)
        q, k, v = qkv[0], qkv[1], qkv[2]
        scores = jnp.einsum("bhqd,bhkd->bhqk", q, k) * (Dh ** -0.5)
        p = _softmax(scores, axis=-1)
        o = jnp.einsum("bhqk,bhkd->bhqd", p, v)
        return (lambda x, *d: x.transpose(*d))(o, 0, 2, 1, 3).reshape(B, S, D) @ wo

    def _B_ref(x, w1, b1, w2, b2):
        B, S, D = x.shape
        h = _layernorm(x, axis=-1)
        u = jnp.einsum("bsd,sf->bdf", h, w1) + b1
        u = _gelu(u)
        y = jnp.einsum("bdf,fs->bds", u, w2) + b2
        return (lambda x, *d: x.transpose(*d))(y, 0, 2, 1)

    x = A_x
    h = x + _A_ref(_layernorm(x, axis=-1), A_wqkv, A_wo)
    h2 = h + _B_ref(_layernorm(h, axis=-1), B_w1, B_b1, B_w2, B_b2)
    return h2
```

```python
import math

import jax
import jax.numpy as jnp
import jax.experimental.pallas as pl
import jax.experimental.pallas.tpu as pltpu

S = 2048
D = 448
H = 16
DH = 28
HP = 32
DP = H * HP
F = 1792
EPS = 1e-5

TQ = 512
KC = 128
SPB = 2
RC = 256
CC = 512
FC = 256
YC = 256

NT = (((1,), (1,)), ((), ()))


def _kernel(x_ref, wqkv_ref, wo_ref, b1_ref, b2_ref, w1_hbm, w2_hbm, o_ref,
            w1_v, w2_v, sems, tmp_ref, wt_ref, wot_ref,
            k_ref, qt_ref, vt_ref, ot_ref, s0_ref, s1_ref, m0_ref, m1_ref,
            ht_ref, ln2_ref, u_ref):
    f32 = jnp.float32
    bf16 = jnp.bfloat16

    cp1 = pltpu.make_async_copy(w1_hbm, w1_v, sems.at[0])
    cp2 = pltpu.make_async_copy(w2_hbm, w2_v, sems.at[1])
    cp1.start()
    cp2.start()

    tmp_ref[...] = wqkv_ref[...].astype(f32).T
    zpad = jnp.zeros((HP - DH, D), f32)
    for hh in range(3 * H):
        blk = tmp_ref[DH * hh:DH * hh + DH, :]
        wt_ref[HP * hh:HP * hh + HP, :] = jnp.concatenate([blk, zpad], axis=0).astype(bf16)
    tmp_ref[0:D, :] = wo_ref[...].astype(f32)
    blks = []
    for hh in range(H):
        blks.append(tmp_ref[DH * hh:DH * hh + DH, :])
        blks.append(zpad)
    wot_ref[...] = jnp.concatenate(blks, axis=0).T.astype(bf16)

    qscale = (DH ** -0.5) * math.log2(math.e)
    rows = jax.lax.broadcasted_iota(jnp.int32, (DP, RC), 0)
    ones_rows = jnp.where((rows % HP) == DH, 1.0, 0.0).astype(f32)
    for c in range(S // RC):
        sl = slice(c * RC, (c + 1) * RC)
        xx = x_ref[sl, :].astype(f32)
        ht_ref[:, sl] = xx.T
        mu = jnp.mean(xx, axis=-1, keepdims=True)
        dd = xx - mu
        var = jnp.mean(dd * dd, axis=-1, keepdims=True)
        ln = (dd * jax.lax.rsqrt(var + EPS)).astype(bf16)
        kk = jax.lax.dot_general(ln, wt_ref[DP:2 * DP, :], NT, preferred_element_type=f32)
        k_ref[sl, :] = kk.astype(bf16)
        qq = jax.lax.dot_general(wt_ref[0:DP, :], ln, NT, preferred_element_type=f32)
        qt_ref[:, sl] = (qq * qscale).astype(bf16)
        vv = jax.lax.dot_general(wt_ref[2 * DP:3 * DP, :], ln, NT, preferred_element_type=f32)
        vt_ref[:, sl] = (vv + ones_rows).astype(bf16)

    NQ = S // TQ
    NSTEP = H * NQ
    NKC = S // KC
    sbuf = [s0_ref, s1_ref]
    mbuf = [m0_ref, m1_ref]

    def step(t1, slot1, t2, slot2):
        if t1 is not None:
            h = t1 // NQ
            qb = t1 % NQ
            g = h // 4
            j = h % 4
            qcol = pl.ds(pl.multiple_of(qb * TQ, TQ), TQ)
            gsl = pl.ds(pl.multiple_of(g * 128, 128), 128)
            qt_g = qt_ref[gsl, qcol]
            row = jax.lax.broadcasted_iota(jnp.int32, (128, TQ), 0)
            w = jnp.where((row // HP) == j, qt_g, jnp.zeros_like(qt_g))
        if t2 is not None:
            h2 = t2 // NQ
            qb2 = t2 % NQ
            qcol2 = pl.ds(pl.multiple_of(qb2 * TQ, TQ), TQ)
            hsl = pl.ds(pl.multiple_of(h2 * HP, HP), HP)
            m = mbuf[slot2][...]
        mx = None
        o = None
        for c in range(NKC):
            ksl = pl.ds(c * KC, KC)
            if t1 is not None:
                st = jnp.dot(k_ref[ksl, gsl], w, preferred_element_type=f32)
                sbuf[slot1][ksl, :] = st
                cm = jnp.max(st.reshape(KC // 8, 8, TQ), axis=0)
                mx = cm if mx is None else jnp.maximum(mx, cm)
            if t2 is not None:
                p = jnp.exp2(sbuf[slot2][ksl, :] - m).astype(bf16)
                oc = jnp.dot(vt_ref[hsl, ksl], p, preferred_element_type=f32)
                o = oc if o is None else o + oc
        if t1 is not None:
            mbuf[slot1][...] = jnp.max(mx, axis=0, keepdims=True)
        if t2 is not None:
            o = o / o[DH:DH + 1, :]
            ot_ref[hsl, qcol2] = o.astype(bf16)

    step(0, 0, None, None)

    def body(i, carry):
        t = SPB * i
        for u in range(SPB):
            step(t + u + 1, (u + 1) % 2, t + u, u % 2)
        return carry

    jax.lax.fori_loop(0, NSTEP // SPB - 1, body, 0)
    t = NSTEP - SPB
    for u in range(SPB - 1):
        step(t + u + 1, (u + 1) % 2, t + u, u % 2)
    step(None, None, NSTEP - 1, (NSTEP - 1) % 2)

    for c in range(S // CC):
        sl = slice(c * CC, (c + 1) * CC)
        at = jnp.dot(wot_ref[...], ot_ref[:, sl], preferred_element_type=f32)
        hh = ht_ref[:, sl] + at
        ht_ref[:, sl] = hh
        mu = jnp.mean(hh, axis=0, keepdims=True)
        dd = hh - mu
        var = jnp.mean(dd * dd, axis=0, keepdims=True)
        ln2_ref[:, sl] = (dd * jax.lax.rsqrt(var + EPS)).astype(bf16)

    cp1.wait()
    for c in range(F // FC):
        sl = slice(c * FC, (c + 1) * FC)
        uu = jnp.dot(ln2_ref[...], w1_v[:, sl], preferred_element_type=f32)
        uu = uu + b1_ref[:, sl].astype(f32)
        u_ref[:, sl] = jax.nn.gelu(uu, approximate=True).astype(bf16)
    cp2.wait()
    for c in range(S // YC):
        sl = slice(c * YC, (c + 1) * YC)
        yy = jnp.dot(u_ref[...], w2_v[:, sl], preferred_element_type=f32)
        yy = yy + b2_ref[:, sl].astype(f32) + ht_ref[:, sl]
        o_ref[sl, :] = yy.T.astype(o_ref.dtype)


@jax.jit
def pallas_sequential_preLN__mha_block__mixer_token_mlp__prompt_kernel(
    A_x: jax.Array,
    A_wqkv: jax.Array,
    A_wo: jax.Array,
    B_x: jax.Array,
    B_w1: jax.Array,
    B_b1: jax.Array,
    B_w2: jax.Array,
    B_b2: jax.Array,
):
    del B_x
    f32 = jnp.float32
    bf16 = jnp.bfloat16
    x = A_x.reshape(S, D)
    b1 = B_b1.reshape(1, F)
    b2 = B_b2.reshape(1, S)

    vmem = pl.BlockSpec(memory_space=pltpu.VMEM)
    hbm = pl.BlockSpec(memory_space=pl.ANY)
    out = pl.pallas_call(
        _kernel,
        out_shape=jax.ShapeDtypeStruct((S, D), A_x.dtype),
        in_specs=[vmem, vmem, vmem, vmem, vmem, hbm, hbm],
        out_specs=vmem,
        scratch_shapes=[
            pltpu.VMEM((S, F), bf16),
            pltpu.VMEM((F, S), bf16),
            pltpu.SemaphoreType.DMA((2,)),
            pltpu.VMEM((3 * D, D), f32),
            pltpu.VMEM((3 * DP, D), bf16),
            pltpu.VMEM((D, DP), bf16),
            pltpu.VMEM((S, DP), bf16),
            pltpu.VMEM((DP, S), bf16),
            pltpu.VMEM((DP, S), bf16),
            pltpu.VMEM((DP, S), bf16),
            pltpu.VMEM((S, TQ), f32),
            pltpu.VMEM((S, TQ), f32),
            pltpu.VMEM((1, TQ), f32),
            pltpu.VMEM((1, TQ), f32),
            pltpu.VMEM((D, S), f32),
            pltpu.VMEM((D, S), bf16),
            pltpu.VMEM((D, F), bf16),
        ],
        compiler_params=pltpu.CompilerParams(vmem_limit_bytes=100 * 1024 * 1024),
    )(x, A_wqkv, A_wo, b1, b2, B_w1, B_w2)
    return out.reshape(1, S, D)
```

```python
import math

import jax
import jax.numpy as jnp
import jax.experimental.pallas as pl
import jax.experimental.pallas.tpu as pltpu

S = 2048
D = 448
H = 16
DH = 28
HP = 32
DP = H * HP
GH = 4
GW = GH * DH
NG = H // GH
F = 1792
EPS = 1e-5

TQ = 512
KC = 128
SPB = 2
RC = 256
CC = 512
FC = 256
YC = 256


def _layernorm_rows(xx):
    mu = jnp.mean(xx, axis=0, keepdims=True)
    dd = xx - mu
    var = jnp.mean(dd * dd, axis=0, keepdims=True)
    return dd * jax.lax.rsqrt(var + EPS)


def _kernel(xt_hbm, wqkv_hbm, wo_hbm, b1_ref, b2_ref, w1_hbm, w2_hbm, o_hbm,
            xt_v, wqkv_v, wo_v, w1_v, w2_v, out_v, sems, osems,
            tmp_ref, wt_ref, wot_ref,
            k_ref, qt_ref, vt_ref, ot_ref, s0_ref, s1_ref, m0_ref, m1_ref,
            ht_ref, ln2_ref, u_ref):
    f32 = jnp.float32
    bf16 = jnp.bfloat16

    cp_w = pltpu.make_async_copy(wqkv_hbm, wqkv_v, sems.at[0])
    cp_x = pltpu.make_async_copy(xt_hbm, xt_v, sems.at[1])
    cp_o = pltpu.make_async_copy(wo_hbm, wo_v, sems.at[2])
    cp1 = pltpu.make_async_copy(w1_hbm, w1_v, sems.at[3])
    cp2 = pltpu.make_async_copy(w2_hbm, w2_v, sems.at[4])
    cp_w.start()
    cp_x.start()
    cp_o.start()

    cp_w.wait()
    tmp_ref[...] = wqkv_v[...].astype(f32).T
    wt_ref[0:2 * D, :] = tmp_ref[0:2 * D, :].astype(bf16)
    zpad = jnp.zeros((HP - DH, D), f32)
    for hh in range(H):
        blk = tmp_ref[2 * D + DH * hh:2 * D + DH * hh + DH, :]
        wt_ref[2 * D + HP * hh:2 * D + HP * hh + HP, :] = (
            jnp.concatenate([blk, zpad], axis=0).astype(bf16))
    cp_x.wait()
    cp_o.wait()
    cp1.start()
    cp2.start()
    tmp_ref[0:D, :] = wo_v[...].astype(f32)
    blks = []
    for hh in range(H):
        blks.append(tmp_ref[DH * hh:DH * hh + DH, :])
        blks.append(zpad)
    wot_ref[...] = jnp.concatenate(blks, axis=0).T.astype(bf16)

    qscale = (DH ** -0.5) * math.log2(math.e)
    rows = jax.lax.broadcasted_iota(jnp.int32, (DP, RC), 0)
    ones_rows = jnp.where((rows % HP) == DH, 1.0, 0.0).astype(f32)
    zgrp = jnp.zeros((128 - GW, RC), f32)
    for c in range(S // RC):
        sl = slice(c * RC, (c + 1) * RC)
        ln = _layernorm_rows(xt_v[:, sl].astype(f32)).astype(bf16)
        qkv = jnp.dot(wt_ref[...], ln, preferred_element_type=f32)
        for g in range(NG):
            qg = qkv[GW * g:GW * g + GW, :] * qscale
            qt_ref[128 * g:128 * g + 128, sl] = jnp.concatenate([qg, zgrp], axis=0).astype(bf16)
            kg = jnp.concatenate([qkv[D + GW * g:D + GW * g + GW, :], zgrp], axis=0)
            k_ref[sl, 128 * g:128 * g + 128] = kg.T.astype(bf16)
        vt_ref[:, sl] = (qkv[2 * D:2 * D + DP, :] + ones_rows).astype(bf16)

    NQ = S // TQ
    NSTEP = H * NQ
    NKC = S // KC
    sbuf = [s0_ref, s1_ref]
    mbuf = [m0_ref, m1_ref]

    def step(t1, slot1, t2, slot2):
        if t1 is not None:
            h = t1 // NQ
            qb = t1 % NQ
            g = h // GH
            j = h % GH
            qcol = pl.ds(pl.multiple_of(qb * TQ, TQ), TQ)
            gsl = pl.ds(pl.multiple_of(g * 128, 128), 128)
            qt_g = qt_ref[gsl, qcol]
            row = jax.lax.broadcasted_iota(jnp.int32, (128, TQ), 0)
            lo = j * DH
            w = jnp.where((row >= lo) & (row < lo + DH), qt_g, jnp.zeros_like(qt_g))
        if t2 is not None:
            h2 = t2 // NQ
            qb2 = t2 % NQ
            qcol2 = pl.ds(pl.multiple_of(qb2 * TQ, TQ), TQ)
            hsl = pl.ds(pl.multiple_of(h2 * HP, HP), HP)
            m = mbuf[slot2][...]
        mx = None
        o = None
        for c in range(NKC):
            ksl = pl.ds(c * KC, KC)
            if t1 is not None:
                st = jnp.dot(k_ref[ksl, gsl], w, preferred_element_type=f32)
                sbuf[slot1][ksl, :] = st
                cm = jnp.max(st.reshape(KC // 8, 8, TQ), axis=0)
                mx = cm if mx is None else jnp.maximum(mx, cm)
            if t2 is not None:
                p = jnp.exp2(sbuf[slot2][ksl, :] - m).astype(bf16)
                oc = jnp.dot(vt_ref[hsl, ksl], p, preferred_element_type=f32)
                o = oc if o is None else o + oc
        if t1 is not None:
            mbuf[slot1][...] = jnp.max(mx, axis=0, keepdims=True)
        if t2 is not None:
            o = o / o[DH:DH + 1, :]
            ot_ref[hsl, qcol2] = o.astype(bf16)

    step(0, 0, None, None)

    def body(i, carry):
        t = SPB * i
        for u in range(SPB):
            step(t + u + 1, (u + 1) % 2, t + u, u % 2)
        return carry

    jax.lax.fori_loop(0, NSTEP // SPB - 1, body, 0)
    t = NSTEP - SPB
    for u in range(SPB - 1):
        step(t + u + 1, (u + 1) % 2, t + u, u % 2)
    step(None, None, NSTEP - 1, (NSTEP - 1) % 2)

    for c in range(S // CC):
        sl = slice(c * CC, (c + 1) * CC)
        at = jnp.dot(wot_ref[...], ot_ref[:, sl], preferred_element_type=f32)
        hh = xt_v[:, sl].astype(f32) + at
        ht_ref[:, sl] = hh
        ln2_ref[:, sl] = _layernorm_rows(hh).astype(bf16)

    b1 = b1_ref[...].astype(f32)
    b2 = b2_ref[...].astype(f32)
    cp1.wait()
    for c in range(F // FC):
        sl = slice(c * FC, (c + 1) * FC)
        uu = jnp.dot(ln2_ref[...], w1_v[:, sl], preferred_element_type=f32)
        uu = uu + b1[:, sl]
        u_ref[:, sl] = jax.nn.gelu(uu, approximate=True).astype(bf16)
    cp2.wait()
    out_cps = []
    for c in range(S // YC):
        sl = slice(c * YC, (c + 1) * YC)
        yy = jnp.dot(u_ref[...], w2_v[:, sl], preferred_element_type=f32)
        yy = yy + b2[:, sl] + ht_ref[:, sl]
        out_v[:, sl] = yy.astype(out_v.dtype)
        cp = pltpu.make_async_copy(out_v.at[:, sl], o_hbm.at[:, sl], osems.at[c])
        cp.start()
        out_cps.append(cp)
    for cp in out_cps:
        cp.wait()


@jax.jit
def pallas_sequential_preLN__mha_block__mixer_token_mlp__prompt_kernel(
    A_x: jax.Array,
    A_wqkv: jax.Array,
    A_wo: jax.Array,
    B_x: jax.Array,
    B_w1: jax.Array,
    B_b1: jax.Array,
    B_w2: jax.Array,
    B_b2: jax.Array,
):
    del B_x
    f32 = jnp.float32
    bf16 = jnp.bfloat16
    xt = A_x.reshape(S, D).T
    b1 = B_b1.reshape(1, F)
    b2 = B_b2.reshape(1, S)

    vmem = pl.BlockSpec(memory_space=pltpu.VMEM)
    hbm = pl.BlockSpec(memory_space=pl.ANY)
    out_t = pl.pallas_call(
        _kernel,
        out_shape=jax.ShapeDtypeStruct((D, S), A_x.dtype),
        in_specs=[hbm, hbm, hbm, vmem, vmem, hbm, hbm],
        out_specs=hbm,
        scratch_shapes=[
            pltpu.VMEM((D, S), bf16),
            pltpu.VMEM((D, 3 * D), bf16),
            pltpu.VMEM((D, D), bf16),
            pltpu.VMEM((S, F), bf16),
            pltpu.VMEM((F, S), bf16),
            pltpu.VMEM((D, S), bf16),
            pltpu.SemaphoreType.DMA((5,)),
            pltpu.SemaphoreType.DMA((S // YC,)),
            pltpu.VMEM((3 * D, D), f32),
            pltpu.VMEM((2 * D + DP, D), bf16),
            pltpu.VMEM((D, DP), bf16),
            pltpu.VMEM((S, NG * 128), bf16),
            pltpu.VMEM((NG * 128, S), bf16),
            pltpu.VMEM((DP, S), bf16),
            pltpu.VMEM((DP, S), bf16),
            pltpu.VMEM((S, TQ), f32),
            pltpu.VMEM((S, TQ), f32),
            pltpu.VMEM((1, TQ), f32),
            pltpu.VMEM((1, TQ), f32),
            pltpu.VMEM((D, S), f32),
            pltpu.VMEM((D, S), bf16),
            pltpu.VMEM((D, F), bf16),
        ],
        compiler_params=pltpu.CompilerParams(vmem_limit_bytes=100 * 1024 * 1024),
    )(xt, A_wqkv, A_wo, b1, b2, B_w1, B_w2)
    return out_t.T.reshape(1, S, D)
```

```python
import math

import jax
import jax.numpy as jnp
import jax.experimental.pallas as pl
import jax.experimental.pallas.tpu as pltpu

S = 2048
D = 448
H = 16
DH = 28
HP = 32
DP = H * HP
GH = 4
NG = H // GH
F = 1792
EPS = 1e-5

TQ = 512
KC = 256
SPB = 16
SKEW = 1
RC = 256
CC = 512
FC = 256
YC = 256
NXC = S // RC
NOC = S // YC
NWB = 4
NQ = S // TQ
NSTEP = H * NQ
NKC = S // KC

L_LO = 2.0 ** -40
L_HI = 2.0 ** 20


def _layernorm_rows(xx):
    mu = jnp.mean(xx, axis=0, keepdims=True)
    dd = xx - mu
    var = jnp.mean(dd * dd, axis=0, keepdims=True)
    return dd * jax.lax.rsqrt(var + EPS)


def _kernel(xt_hbm, wqkv_hbm, wo_hbm, b1_hbm, b2_hbm, w1_hbm, w2_hbm, o_hbm,
            xt_v, wqkv_v, wo_v, b1_v, b2_v, w1_v, w2_v, out_v, sems, wsems, xsems, osems,
            tmp_ref, wt_ref, wot_ref,
            k_ref, qp_ref, vt_ref, ot_ref, nq_ref, ok_ref, ocar_ref, pc0_ref, pc1_ref,
            s_ref, ht_ref, ln2_ref, u_ref):
    f32 = jnp.float32
    bf16 = jnp.bfloat16
    pcar = [pc0_ref, pc1_ref]

    cp_w = [
        pltpu.make_async_copy(wqkv_hbm.at[r * (D // NWB):(r + 1) * (D // NWB), :],
                              wqkv_v.at[r * (D // NWB):(r + 1) * (D // NWB), :], wsems.at[r])
        for r in range(NWB)
    ]
    cp_o = pltpu.make_async_copy(wo_hbm, wo_v, sems.at[1])
    cp_b1 = pltpu.make_async_copy(b1_hbm, b1_v, sems.at[2])
    cp_b2 = pltpu.make_async_copy(b2_hbm, b2_v, sems.at[3])
    cp1 = pltpu.make_async_copy(w1_hbm, w1_v, sems.at[4])
    cp2 = pltpu.make_async_copy(w2_hbm, w2_v, sems.at[5])
    cp_x = [
        pltpu.make_async_copy(xt_hbm.at[:, c * RC:(c + 1) * RC],
                              xt_v.at[:, c * RC:(c + 1) * RC], xsems.at[c])
        for c in range(NXC)
    ]
    for cp in cp_w:
        cp.start()
    cp_x[0].start()

    for cp in cp_w:
        cp.wait()
    cp_x[0].wait()
    cp_x[1].start()
    cp_x[2].start()
    cp_x[3].start()

    qscale = (DH ** -0.5) * math.log2(math.e)
    prow = jax.lax.broadcasted_iota(jnp.int32, (HP - DH, RC), 0)
    pad_zero = jnp.zeros((HP - DH, RC), f32)
    pad_one = jnp.where(prow == 0, 1.0, 0.0).astype(f32)

    def ln1(c):
        return _layernorm_rows(xt_v[:, c * RC:(c + 1) * RC].astype(f32)).astype(bf16)

    ln = ln1(0)
    kmax = None
    for c in range(NXC):
        sl = slice(c * RC, (c + 1) * RC)
        if c == 1:
            cp_x[1].wait()
            cp_x[2].wait()
            cp_x[3].wait()
            for cc in range(4, NXC):
                cp_x[cc].start()
            cp_o.start()
            cp_b1.start()
            cp_b2.start()
            ln = ln1(1)
        if c == 3:
            for cc in range(4, NXC):
                cp_x[cc].wait()
            cp_o.wait()
        if c == 0:
            qkv = jax.lax.dot_general(wqkv_v[...], ln, (((0,), (0,)), ((), ())),
                                      preferred_element_type=f32)
            wt_ref[...] = wqkv_v[...].astype(f32).T.astype(bf16)
        else:
            qkv = jnp.dot(wt_ref[...], ln, preferred_element_type=f32)
        if 1 < c + 1 < NXC:
            ln = ln1(c + 1)
        nq_rows = []
        nk_rows = []
        for g in range(NG):
            kblks = []
            for j in range(GH):
                hh = g * GH + j
                qf = qkv[DH * hh:DH * hh + DH, :] * qscale
                nq_rows.append(jnp.sum(qf * qf, axis=0, keepdims=True))
                qp_ref[hh, :, sl] = jnp.concatenate([qf, pad_zero], axis=0).astype(bf16)
                kf = qkv[D + DH * hh:D + DH * hh + DH, :]
                nk_rows.append(jnp.sum(kf * kf, axis=0, keepdims=True))
                kblks += [kf, pad_one]
                v = qkv[2 * D + DH * hh:2 * D + DH * hh + DH, :]
                vt_ref[hh, :, sl] = jnp.concatenate([v, pad_one], axis=0).astype(bf16)
            kt = jnp.concatenate(kblks, axis=0).T.astype(bf16)
            k_ref[g, c * (RC // 2):(c + 1) * (RC // 2), :] = pltpu.bitcast(kt, jnp.uint32)
        nq_ref[:, sl] = jnp.sqrt(jnp.concatenate(nq_rows, axis=0))
        nk = jnp.concatenate(nk_rows, axis=0)
        kmax = nk if kmax is None else jnp.maximum(kmax, nk)
        if c == 4:
            tmp_ref[...] = wo_v[...].astype(f32)
            zpad = jnp.zeros((HP - DH, D), f32)
            blks = []
            for hh in range(H):
                blks.append(tmp_ref[DH * hh:DH * hh + DH, :])
                blks.append(zpad)
            wot_ref[...] = pltpu.bitcast(jnp.concatenate(blks, axis=0).T.astype(bf16), jnp.uint32)

    kmax = jnp.sqrt(jnp.max(kmax, axis=1, keepdims=True)) * (-(1.0 + 2.0 ** -6))
    nq_ref[...] = nq_ref[...] * kmax

    def idx(t):
        qb, h = t
        return h, pl.ds(pl.multiple_of(qb * TQ, TQ), TQ), pl.ds(pl.multiple_of(h * HP, HP), HP)

    def weights(t, with_bound):
        h, qcol, _ = idx(t)
        qp = qp_ref[h, :, qcol]
        j = h % GH
        if with_bound:
            assert isinstance(h, int)
            nb = jnp.broadcast_to(nq_ref[h:h + 1, qcol], (HP, TQ)).astype(bf16)
            r32 = jax.lax.broadcasted_iota(jnp.int32, (HP, TQ), 0)
            qp = jnp.where(r32 == DH, nb, qp)
            zero = jnp.zeros_like(qp)
            return jnp.concatenate([qp if jj == j else zero for jj in range(GH)], axis=0)
        q4 = jnp.concatenate([qp] * GH, axis=0)
        row = jax.lax.broadcasted_iota(jnp.int32, (128, TQ), 0)
        return jnp.where((row // HP) == j, q4, jnp.zeros_like(q4))

    def pv(t, c, p, o):
        h, _, _ = idx(t)
        oc = jnp.dot(vt_ref[h, :, pl.ds(c * KC, KC)], p, preferred_element_type=f32)
        return oc if o is None else o + oc

    def finalize(t, o, check):
        _, qcol, hsl = idx(t)
        l = o[DH:DH + 1, :]
        if check:
            good = jnp.where((l >= L_LO) & (l <= L_HI), 1.0, 0.0)
            ok_ref[...] = jnp.minimum(ok_ref[...], good)
        ot_ref[hsl, qcol] = (o / l).astype(bf16)

    def body(i, carry):
        @pl.when(i == 0)
        def _():
            cp1.start()
            cp2.start()

        tprev = (jnp.maximum(i - 1, 0), H - 1)
        ps = {}
        o = ocar_ref[...]
        for n in range(SPB * NKC):
            u, c = divmod(n, NKC)
            if c == 0:
                w = weights((i, u), True)
                g = u // GH
            kk = pltpu.bitcast(k_ref[g, pl.ds(c * (KC // 2), KC // 2), :], bf16)
            st = jnp.dot(kk, w, preferred_element_type=f32)
            ps[n] = jnp.exp2(st).astype(bf16)
            m = n - SKEW
            if m < 0:
                tm, cm, p = tprev, NKC + m, pcar[n][...]
            else:
                tm, cm, p = (i, m // NKC), m % NKC, ps.pop(m)
            o = pv(tm, cm, p, o)
            if cm == NKC - 1:
                finalize(tm, o, True)
                o = None
        for s in range(SKEW):
            pcar[s][...] = ps.pop(SPB * NKC - SKEW + s)
        ocar_ref[...] = o
        return carry

    for s in range(SKEW):
        pcar[s][...] = jnp.zeros((KC, TQ), bf16)
    ocar_ref[...] = jnp.ones((HP, TQ), f32)
    ok_ref[...] = jnp.ones((1, TQ), f32)
    assert SPB == H
    jax.lax.fori_loop(0, NQ, body, 0)
    cp_b1.wait()
    cp_b2.wait()
    cp1.wait()
    cp2.wait()
    o = ocar_ref[...]
    for s in range(SKEW):
        o = pv((NQ - 1, H - 1), NKC - SKEW + s, pcar[s][...], o)
    finalize((NQ - 1, H - 1), o, True)

    def out_projection():
        for c in range(S // CC):
            sl = slice(c * CC, (c + 1) * CC)
            at = jnp.dot(pltpu.bitcast(wot_ref[...], bf16), ot_ref[:, sl], preferred_element_type=f32)
            hh = xt_v[:, sl].astype(f32) + at
            ht_ref[:, sl] = hh
            ln2_ref[:, sl] = pltpu.bitcast(_layernorm_rows(hh).astype(bf16), jnp.uint32)

    all_ok = jnp.min(ok_ref[...])
    out_projection()

    for c in range(F // FC):
        sl = slice(c * FC, (c + 1) * FC)
        uu = jnp.dot(pltpu.bitcast(ln2_ref[...], bf16), w1_v[:, sl], preferred_element_type=f32)
        uu = uu + b1_v[sl].astype(f32).reshape(1, FC)
        u_ref[:, sl] = pltpu.bitcast(jax.nn.gelu(uu, approximate=True).astype(bf16), jnp.uint32)
    out_cps = []
    for c in range(NOC):
        sl = slice(c * YC, (c + 1) * YC)
        yy = jnp.dot(pltpu.bitcast(u_ref[...], bf16), w2_v[:, sl], preferred_element_type=f32)
        yy = yy + b2_v[sl].astype(f32).reshape(1, YC) + ht_ref[:, sl]
        out_v[:, sl] = yy.astype(out_v.dtype)
        cp = pltpu.make_async_copy(out_v.at[:, sl], o_hbm.at[:, sl], osems.at[c])
        cp.start()
        out_cps.append(cp)

    @pl.when(all_ok < 0.5)
    def _():
        for cp in out_cps:
            cp.wait()

        def slow_step(tt, carry):
            t = (tt % NQ, tt // NQ)
            h, _, _ = idx(t)
            g = h // GH
            w = weights(t, False)

            def pass1(c, mx):
                ksl = pl.ds(pl.multiple_of(c * KC, KC), KC)
                kk = pltpu.bitcast(k_ref[g, pl.ds(pl.multiple_of(c * (KC // 2), 8), KC // 2), :], bf16)
                st = jnp.dot(kk, w, preferred_element_type=f32)
                s_ref[ksl, :] = st
                return jnp.maximum(mx, jnp.max(st, axis=0, keepdims=True))

            mx = jax.lax.fori_loop(0, NKC, pass1, jnp.full((1, TQ), -jnp.inf, f32))

            def pass2(c, o):
                ksl = pl.ds(pl.multiple_of(c * KC, KC), KC)
                p = jnp.exp2(s_ref[ksl, :] - mx).astype(bf16)
                return o + jnp.dot(vt_ref[h, :, ksl], p, preferred_element_type=f32)

            o = jax.lax.fori_loop(0, NKC, pass2, jnp.zeros((HP, TQ), f32))
            finalize(t, o, False)
            return carry

        jax.lax.fori_loop(0, NSTEP, slow_step, 0)

        def slow_proj(c, carry):
            sl = pl.ds(pl.multiple_of(c * 128, 128), 128)
            at = jnp.dot(pltpu.bitcast(wot_ref[...], bf16), ot_ref[:, sl], preferred_element_type=f32)
            hh = xt_v[:, sl].astype(f32) + at
            ht_ref[:, sl] = hh
            ln2_ref[:, sl] = pltpu.bitcast(_layernorm_rows(hh).astype(bf16), jnp.uint32)
            return carry

        jax.lax.fori_loop(0, S // 128, slow_proj, 0)

        def slow_u(c, carry):
            sl = pl.ds(pl.multiple_of(c * FC, FC), FC)
            uu = jnp.dot(pltpu.bitcast(ln2_ref[...], bf16), w1_v[:, sl], preferred_element_type=f32)
            uu = uu + b1_v[sl].astype(f32).reshape(1, FC)
            u_ref[:, sl] = pltpu.bitcast(jax.nn.gelu(uu, approximate=True).astype(bf16), jnp.uint32)
            return carry

        jax.lax.fori_loop(0, F // FC, slow_u, 0)

        def slow_y(c, carry):
            sl = pl.ds(pl.multiple_of(c * YC, YC), YC)
            yy = jnp.dot(pltpu.bitcast(u_ref[...], bf16), w2_v[:, sl], preferred_element_type=f32)
            yy = yy + b2_v[sl].astype(f32).reshape(1, YC) + ht_ref[:, sl]
            out_v[:, sl] = yy.astype(out_v.dtype)
            return carry

        jax.lax.fori_loop(0, NOC, slow_y, 0)
        for cp in out_cps:
            cp.start()

    for cp in out_cps:
        cp.wait()


@jax.jit
def pallas_sequential_preLN__mha_block__mixer_token_mlp__prompt_kernel(
    A_x: jax.Array,
    A_wqkv: jax.Array,
    A_wo: jax.Array,
    B_x: jax.Array,
    B_w1: jax.Array,
    B_b1: jax.Array,
    B_w2: jax.Array,
    B_b2: jax.Array,
):
    del B_x
    f32 = jnp.float32
    bf16 = jnp.bfloat16
    xt = A_x.reshape(S, D).T

    hbm = pl.BlockSpec(memory_space=pl.ANY)
    out_t = pl.pallas_call(
        _kernel,
        out_shape=jax.ShapeDtypeStruct((D, S), A_x.dtype),
        in_specs=[hbm] * 7,
        out_specs=hbm,
        scratch_shapes=[
            pltpu.VMEM((D, S), bf16),
            pltpu.VMEM((D, 3 * D), bf16),
            pltpu.VMEM((D, D), bf16),
            pltpu.VMEM((F,), bf16),
            pltpu.VMEM((S,), bf16),
            pltpu.VMEM((S, F), bf16),
            pltpu.VMEM((F, S), bf16),
            pltpu.VMEM((D, S), bf16),
            pltpu.SemaphoreType.DMA((6,)),
            pltpu.SemaphoreType.DMA((NWB,)),
            pltpu.SemaphoreType.DMA((NXC,)),
            pltpu.SemaphoreType.DMA((NOC,)),
            pltpu.VMEM((D, D), f32),
            pltpu.VMEM((3 * D, D), bf16),
            pltpu.VMEM((D // 2, DP), jnp.uint32),
            pltpu.VMEM((NG, S // 2, 128), jnp.uint32),
            pltpu.VMEM((H, HP, S), bf16),
            pltpu.VMEM((H, HP, S), bf16),
            pltpu.VMEM((DP, S), bf16),
            pltpu.VMEM((H, S), f32),
            pltpu.VMEM((1, TQ), f32),
            pltpu.VMEM((HP, TQ), f32),
            pltpu.VMEM((KC, TQ), bf16),
            pltpu.VMEM((KC, TQ), bf16),
            pltpu.VMEM((S, TQ), f32),
            pltpu.VMEM((D, S), f32),
            pltpu.VMEM((D // 2, S), jnp.uint32),
            pltpu.VMEM((D // 2, F), jnp.uint32),
        ],
        compiler_params=pltpu.CompilerParams(vmem_limit_bytes=100 * 1024 * 1024),
    )(xt, A_wqkv, A_wo, B_b1, B_b2, B_w1, B_w2)
    return out_t.T.reshape(1, S, D)
```
